```python
import os as _os
_os.environ.setdefault("JAX_PLATFORMS", "cpu")
import jax
import jax.numpy as jnp

def _softmax(x, axis=-1):
    return jax.nn.softmax(x, axis=axis)
def _gelu(x):
    return jax.nn.gelu(x, approximate=True)
def _silu(x):
    return jax.nn.silu(x)
def _sigmoid(x):
    return jax.nn.sigmoid(x)
def _layernorm(x, axis=-1, eps=1e-5):
    m = jnp.mean(x, axis=axis, keepdims=True)
    v = jnp.var(x, axis=axis, keepdims=True)
    return (x - m) / jnp.sqrt(v + eps)
def _scatter_add(tgt, idx, src, axis=0):
    return tgt.at[idx].add(src)
def _segment_sum(src, seg, n):
    return jax.ops.segment_sum(src, seg, n)
class _Rng:
    def __init__(self, key):
        self._k = key
    def _next(self):
        self._k, sub = jax.random.split(self._k)
        return sub
    def normal(self, shape):
        return jax.random.normal(self._next(), shape, dtype=jnp.bfloat16)
    def randint(self, lo, hi, shape):
        return jax.random.randint(self._next(), shape, lo, hi, dtype=jnp.int32)
    def uniform(self, shape, lo=0.0, hi=1.0):
        return jax.random.uniform(self._next(), shape, jnp.bfloat16, lo, hi)
    def permutation(self, n):
        return jax.random.permutation(self._next(), n)


kernel_name = 'sequential_preLN__spectral_gfnet__glu_gated_bilinear__prompt'

def setup_inputs():
    _rng = _Rng(jax.random.key(int.from_bytes(__import__("os").urandom(4), "little")))
    _w = (lambda a: (lambda t: t.astype(jnp.bfloat16) if jnp.issubdtype(t.dtype, jnp.floating) else t)(jnp.asarray(a)))
    def _A_setup():
        B, S, D = 1, 2048, 448
        Df = D // 2 + 1
        return {
            "x": _w((lambda *s: _rng.normal(s) * 0.05)(B, S, D)),
            "w_r": _w((lambda *s: _rng.normal(s) * 0.2)(S, Df) * 0.02),
            "w_i": _w((lambda *s: _rng.normal(s) * 0.2)(S, Df) * 0.02),
        }
    _A_in = _A_setup()

    def _B_setup():
        B, S, D, F = 1, 2048, 448, 1792
        return {
            "x": _w((lambda *s: _rng.normal(s) * 0.05)(B, S, D)),
            "w_gate": _w((lambda *s: _rng.normal(s) * 0.05)(D, F) * (D ** -0.5)),
            "w_up": _w((lambda *s: _rng.normal(s) * 0.05)(D, F) * (D ** -0.5)),
            "w_down": _w((lambda *s: _rng.normal(s) * 0.05)(F, D) * (F ** -0.5)),
        }
    _B_in = _B_setup()

    return {
        "A_x": _A_in["x"],
        "A_w_r": _A_in["w_r"],
        "A_w_i": _A_in["w_i"],
        "B_x": _B_in["x"],
        "B_w_gate": _B_in["w_gate"],
        "B_w_up": _B_in["w_up"],
        "B_w_down": _B_in["w_down"],
    }

def reference(A_x, A_w_r, A_w_i, B_x, B_w_gate, B_w_up, B_w_down):
    def _A_ref(x, w_r, w_i):
        B, S, D = x.shape
        X = (lambda x, axes=(-2,-1): jnp.fft.rfft2(x.astype(jnp.float32), axes=axes))(x, axes=(-2, -1))
        W = w_r + 1j * w_i
        X = X * W
        y = (lambda x, s, axes=(-2,-1): jnp.fft.irfft2(x, s=s, axes=axes).astype(jnp.bfloat16))(X, (S, D), axes=(-2, -1))
        return y

    def _B_ref(x, w_gate, w_up, w_down):
        g = jnp.einsum("bsd,df->bsf", x, w_gate)
        u = jnp.einsum("bsd,df->bsf", x, w_up)
        h = g * u
        return jnp.einsum("bsf,fd->bsd", h, w_down)

    x = A_x
    h = x + _A_ref(_layernorm(x, axis=-1), A_w_r, A_w_i)
    h2 = h + _B_ref(_layernorm(h, axis=-1), B_w_gate, B_w_up, B_w_down)
    return h2
```

```python
import math

import numpy as np
import jax
import jax.numpy as jnp
import jax.experimental.pallas as pl
import jax.experimental.pallas.tpu as pltpu

S = 2048
D = 448
F = 1792
DF = D // 2 + 1
KP = 256
NA = 16
NB = 128
EPS = 1e-5
FFN_ROWS = 512


def _constants():
    d = np.arange(D)[:, None].astype(np.float64)
    k = np.arange(KP)[None, :].astype(np.float64)
    valid = (np.arange(KP) < DF)[None, :]
    ang = 2.0 * np.pi * d * k / D
    fd = np.concatenate(
        [np.where(valid, np.cos(ang), 0.0), np.where(valid, -np.sin(ang), 0.0)], axis=1
    )

    b = np.arange(NB).astype(np.float64)
    angb = 2.0 * np.pi * b[:, None] * b[None, :] / NB
    fr, fi = np.cos(angb), -np.sin(angb)
    ff = np.block([[fr, -fi], [fi, fr]])
    fv = np.block([[fr, fi], [-fi, fr]])

    fa = np.arange(NA).astype(np.float64)
    angt = 2.0 * np.pi * b[None, :] * fa[:, None] / S
    twr = np.broadcast_to(np.cos(angt)[:, :, None], (NA, NB, 128)).copy()
    twi = np.broadcast_to(-np.sin(angt)[:, :, None], (NA, NB, 128)).copy()

    ck = np.where((np.arange(KP) == 0) | (np.arange(KP) == D // 2), 1.0, 2.0)
    ck = np.where(np.arange(KP) < DF, ck, 0.0)[:, None]
    scale = 1.0 / (D * S)
    angg = 2.0 * np.pi * np.arange(KP)[:, None] * np.arange(D)[None, :] / D
    g = np.concatenate([ck * np.cos(angg) * scale, -ck * np.sin(angg) * scale], axis=0)

    return (
        jnp.asarray(fd, jnp.bfloat16),
        jnp.asarray(ff, jnp.bfloat16),
        jnp.asarray(fv, jnp.bfloat16),
        jnp.asarray(twr, jnp.float32),
        jnp.asarray(twi, jnp.float32),
        jnp.asarray(g, jnp.bfloat16),
    )


def _cmul_const(re, im, c, s):
    if abs(c - 1.0) < 1e-12 and abs(s) < 1e-12:
        return re, im
    if abs(c + 1.0) < 1e-12 and abs(s) < 1e-12:
        return -re, -im
    if abs(c) < 1e-12 and abs(s + 1.0) < 1e-12:
        return im, -re
    if abs(c) < 1e-12 and abs(s - 1.0) < 1e-12:
        return -im, re
    return re * c - im * s, re * s + im * c


def _fft_list(xs, sign):
    n = len(xs)
    if n == 1:
        return xs
    ev = _fft_list(xs[0::2], sign)
    od = _fft_list(xs[1::2], sign)
    out = [None] * n
    for k in range(n // 2):
        ang = sign * 2.0 * math.pi * k / n
        tr, ti = _cmul_const(od[k][0], od[k][1], math.cos(ang), math.sin(ang))
        out[k] = (ev[k][0] + tr, ev[k][1] + ti)
        out[k + n // 2] = (ev[k][0] - tr, ev[k][1] - ti)
    return out


def _layernorm(v):
    mu = jnp.mean(v, axis=-1, keepdims=True)
    c = v - mu
    var = jnp.mean(c * c, axis=-1, keepdims=True)
    return c * jax.lax.rsqrt(var + EPS)


def _kernel(x_ref, wr_ref, wi_ref, wg_ref, wu_ref, wd_ref, fd_ref, ff_ref, fv_ref,
            twr_ref, twi_ref, g_ref, o_ref, z_ref, t_ref, h_ref):
    f32 = jnp.float32
    bf16 = jnp.bfloat16

    for a in range(NA):
        xa = x_ref[a * NB:(a + 1) * NB, :].astype(f32)
        xn = _layernorm(xa).astype(bf16)
        z_ref[a] = jnp.dot(xn, fd_ref[...], preferred_element_type=f32)

    xs = [(z_ref[a, :, 0:KP], z_ref[a, :, KP:2 * KP]) for a in range(NA)]
    ys = _fft_list(xs, -1.0)
    for fa in range(NA):
        re, im = ys[fa]
        if fa > 0:
            c = jnp.concatenate([twr_ref[fa]] * 2, axis=1)
            s = jnp.concatenate([twi_ref[fa]] * 2, axis=1)
            re, im = re * c - im * s, re * s + im * c
        t_ref[0:NB, fa * KP:(fa + 1) * KP] = re.astype(bf16)
        t_ref[NB:2 * NB, fa * KP:(fa + 1) * KP] = im.astype(bf16)

    xx = jnp.dot(ff_ref[...], t_ref[...], preferred_element_type=f32)
    xr = xx[0:NB]
    xi = xx[NB:2 * NB]
    wr = wr_ref[...].astype(f32)
    wi = wi_ref[...].astype(f32)
    t_ref[0:NB, :] = (xr * wr - xi * wi).astype(bf16)
    t_ref[NB:2 * NB, :] = (xr * wi + xi * wr).astype(bf16)
    uu = jnp.dot(fv_ref[...], t_ref[...], preferred_element_type=f32)

    xs = []
    for fa in range(NA):
        re = uu[0:NB, fa * KP:(fa + 1) * KP]
        im = uu[NB:2 * NB, fa * KP:(fa + 1) * KP]
        if fa > 0:
            c = jnp.concatenate([twr_ref[fa]] * 2, axis=1)
            s = jnp.concatenate([twi_ref[fa]] * 2, axis=1)
            re, im = re * c + im * s, im * c - re * s
        xs.append((re, im))
    vs = _fft_list(xs, 1.0)

    for a in range(NA):
        v = jnp.concatenate([vs[a][0], vs[a][1]], axis=1).astype(bf16)
        y = jnp.dot(v, g_ref[...], preferred_element_type=f32).astype(bf16)
        h_ref[a * NB:(a + 1) * NB, :] = (x_ref[a * NB:(a + 1) * NB, :] + y)

    for r in range(S // FFN_ROWS):
        h = h_ref[r * FFN_ROWS:(r + 1) * FFN_ROWS, :]
        hn = _layernorm(h.astype(f32)).astype(bf16)
        gg = jnp.dot(hn, wg_ref[...], preferred_element_type=f32).astype(bf16)
        up = jnp.dot(hn, wu_ref[...], preferred_element_type=f32).astype(bf16)
        hh = gg * up
        out = jnp.dot(hh, wd_ref[...], preferred_element_type=f32).astype(bf16)
        o_ref[r * FFN_ROWS:(r + 1) * FFN_ROWS, :] = h + out


@jax.jit
def pallas_sequential_preLN__spectral_gfnet__glu_gated_bilinear__prompt_kernel(
    A_x: jax.Array,
    A_w_r: jax.Array,
    A_w_i: jax.Array,
    B_x: jax.Array,
    B_w_gate: jax.Array,
    B_w_up: jax.Array,
    B_w_down: jax.Array,
):
    x = A_x.reshape(S, D)

    def perm(w):
        w = jnp.pad(w.reshape(NB, NA, DF), ((0, 0), (0, 0), (0, KP - DF)))
        return w.reshape(NB, NA * KP)

    wr = perm(A_w_r)
    wi = perm(A_w_i)
    fd, ff, fv, twr, twi, g = _constants()

    out = pl.pallas_call(
        _kernel,
        out_shape=jax.ShapeDtypeStruct((S, D), jnp.bfloat16),
        scratch_shapes=[
            pltpu.VMEM((NA, NB, 2 * KP), jnp.float32),
            pltpu.VMEM((2 * NB, NA * KP), jnp.bfloat16),
            pltpu.VMEM((S, D), jnp.bfloat16),
        ],
        compiler_params=pltpu.CompilerParams(vmem_limit_bytes=100 * 1024 * 1024),
    )(x, wr, wi, B_w_gate, B_w_up, B_w_down, fd, ff, fv, twr, twi, g)
    return out.reshape(1, S, D)
```

```python
import math

import numpy as np
import jax
import jax.numpy as jnp
import jax.experimental.pallas as pl
import jax.experimental.pallas.tpu as pltpu

S = 2048
D = 448
F = 1792
DF = D // 2 + 1
KP = 256
NA = 16
NB = 128
EPS = 1e-5
FFN_ROWS = 512


def _constants():
    d = np.arange(D)[:, None].astype(np.float64)
    k = np.arange(KP)[None, :].astype(np.float64)
    valid = (np.arange(KP) < DF)[None, :]
    ang = 2.0 * np.pi * d * k / D
    fd = np.concatenate(
        [np.where(valid, np.cos(ang), 0.0), np.where(valid, -np.sin(ang), 0.0)], axis=1
    )

    b = np.arange(NB).astype(np.float64)
    angb = 2.0 * np.pi * b[:, None] * b[None, :] / NB
    fr, fi = np.cos(angb), -np.sin(angb)
    ff = np.block([[fr, -fi], [fi, fr]])
    fv = np.block([[fr, fi], [-fi, fr]])

    fa = np.arange(NA).astype(np.float64)
    angt = 2.0 * np.pi * b[None, :] * fa[:, None] / S
    twr = np.broadcast_to(np.cos(angt)[:, :, None], (NA, NB, 128)).copy()
    twi = np.broadcast_to(-np.sin(angt)[:, :, None], (NA, NB, 128)).copy()

    ck = np.where((np.arange(KP) == 0) | (np.arange(KP) == D // 2), 1.0, 2.0)
    ck = np.where(np.arange(KP) < DF, ck, 0.0)[:, None]
    scale = 1.0 / (D * S)
    angg = 2.0 * np.pi * np.arange(KP)[:, None] * np.arange(D)[None, :] / D
    g = np.concatenate([ck * np.cos(angg) * scale, -ck * np.sin(angg) * scale], axis=0)

    return (
        jnp.asarray(fd, jnp.bfloat16),
        jnp.asarray(ff, jnp.bfloat16),
        jnp.asarray(fv, jnp.bfloat16),
        jnp.asarray(twr, jnp.float32),
        jnp.asarray(twi, jnp.float32),
        jnp.asarray(g, jnp.bfloat16),
    )


def _cmul_const(re, im, c, s):
    if abs(c - 1.0) < 1e-12 and abs(s) < 1e-12:
        return re, im
    if abs(c + 1.0) < 1e-12 and abs(s) < 1e-12:
        return -re, -im
    if abs(c) < 1e-12 and abs(s + 1.0) < 1e-12:
        return im, -re
    if abs(c) < 1e-12 and abs(s - 1.0) < 1e-12:
        return -im, re
    return re * c - im * s, re * s + im * c


def _fft_list(xs, sign):
    n = len(xs)
    if n == 1:
        return xs
    ev = _fft_list(xs[0::2], sign)
    od = _fft_list(xs[1::2], sign)
    out = [None] * n
    for k in range(n // 2):
        ang = sign * 2.0 * math.pi * k / n
        tr, ti = _cmul_const(od[k][0], od[k][1], math.cos(ang), math.sin(ang))
        out[k] = (ev[k][0] + tr, ev[k][1] + ti)
        out[k + n // 2] = (ev[k][0] - tr, ev[k][1] - ti)
    return out


def _layernorm(v):
    mu = jnp.mean(v, axis=-1, keepdims=True)
    c = v - mu
    var = jnp.mean(c * c, axis=-1, keepdims=True)
    return c * jax.lax.rsqrt(var + EPS)


def _kernel(xt_ref, wrt_hbm, wit_hbm, wg_hbm, wu_hbm, wdt_hbm, fd_ref, ff_ref, fv_ref,
            twr_ref, twi_ref, g_ref, o_ref,
            z_ref, t_ref, x_ref, h_ref, wtr_ref, wti_ref, wr_ref, wi_ref, wg_ref, wu_ref, wdt_ref,
            wd_ref, sems):
    f32 = jnp.float32
    bf16 = jnp.bfloat16

    copies = [
        pltpu.make_async_copy(wrt_hbm, wtr_ref, sems.at[0]),
        pltpu.make_async_copy(wit_hbm, wti_ref, sems.at[1]),
        pltpu.make_async_copy(wg_hbm, wg_ref, sems.at[2]),
        pltpu.make_async_copy(wu_hbm, wu_ref, sems.at[3]),
        pltpu.make_async_copy(wdt_hbm, wdt_ref, sems.at[4]),
    ]
    for c in copies:
        c.start()

    x_ref[...] = xt_ref[...].T

    for a in range(NA):
        xa = x_ref[a * NB:(a + 1) * NB, :].astype(f32)
        xn = _layernorm(xa).astype(bf16)
        z_ref[a] = jnp.dot(xn, fd_ref[...], preferred_element_type=f32)

    xs = [(z_ref[a, :, 0:KP], z_ref[a, :, KP:2 * KP]) for a in range(NA)]
    ys = _fft_list(xs, -1.0)
    for fa in range(NA):
        re, im = ys[fa]
        if fa > 0:
            c = jnp.concatenate([twr_ref[fa]] * 2, axis=1)
            s = jnp.concatenate([twi_ref[fa]] * 2, axis=1)
            re, im = re * c - im * s, re * s + im * c
        t_ref[0:NB, fa * KP:(fa + 1) * KP] = re.astype(bf16)
        t_ref[NB:2 * NB, fa * KP:(fa + 1) * KP] = im.astype(bf16)

    xx = jnp.dot(ff_ref[...], t_ref[...], preferred_element_type=f32)
    copies[0].wait()
    copies[1].wait()
    zpad = jnp.zeros((KP - DF, S), f32)
    wr_ref[...] = jnp.concatenate([wtr_ref[...].astype(f32), zpad], axis=0).T.reshape(NB, NA, KP)
    wi_ref[...] = jnp.concatenate([wti_ref[...].astype(f32), zpad], axis=0).T.reshape(NB, NA, KP)
    for fa in range(NA):
        xr = xx[0:NB, fa * KP:(fa + 1) * KP]
        xi = xx[NB:2 * NB, fa * KP:(fa + 1) * KP]
        wr = wr_ref[:, fa, :]
        wi = wi_ref[:, fa, :]
        t_ref[0:NB, fa * KP:(fa + 1) * KP] = (xr * wr - xi * wi).astype(bf16)
        t_ref[NB:2 * NB, fa * KP:(fa + 1) * KP] = (xr * wi + xi * wr).astype(bf16)
    uu = jnp.dot(fv_ref[...], t_ref[...], preferred_element_type=f32)

    xs = []
    for fa in range(NA):
        re = uu[0:NB, fa * KP:(fa + 1) * KP]
        im = uu[NB:2 * NB, fa * KP:(fa + 1) * KP]
        if fa > 0:
            c = jnp.concatenate([twr_ref[fa]] * 2, axis=1)
            s = jnp.concatenate([twi_ref[fa]] * 2, axis=1)
            re, im = re * c + im * s, im * c - re * s
        xs.append((re, im))
    vs = _fft_list(xs, 1.0)

    for a in range(NA):
        v = jnp.concatenate([vs[a][0], vs[a][1]], axis=1).astype(bf16)
        y = jnp.dot(v, g_ref[...], preferred_element_type=f32).astype(bf16)
        h_ref[a * NB:(a + 1) * NB, :] = (x_ref[a * NB:(a + 1) * NB, :] + y)

    copies[2].wait()
    copies[3].wait()
    copies[4].wait()
    wd_ref[...] = wdt_ref[...].T

    for r in range(S // FFN_ROWS):
        h = h_ref[r * FFN_ROWS:(r + 1) * FFN_ROWS, :]
        hn = _layernorm(h.astype(f32)).astype(bf16)
        gg = jnp.dot(hn, wg_ref[...], preferred_element_type=f32).astype(bf16)
        up = jnp.dot(hn, wu_ref[...], preferred_element_type=f32).astype(bf16)
        hh = gg * up
        out = jnp.dot(hh, wd_ref[...], preferred_element_type=f32).astype(bf16)
        o_ref[:, r * FFN_ROWS:(r + 1) * FFN_ROWS] = (h + out).T


@jax.jit
def pallas_sequential_preLN__spectral_gfnet__glu_gated_bilinear__prompt_kernel(
    A_x: jax.Array,
    A_w_r: jax.Array,
    A_w_i: jax.Array,
    B_x: jax.Array,
    B_w_gate: jax.Array,
    B_w_up: jax.Array,
    B_w_down: jax.Array,
):
    xt = A_x.reshape(S, D).T
    fd, ff, fv, twr, twi, g = _constants()
    vm = pl.BlockSpec(memory_space=pltpu.VMEM)
    hbm = pl.BlockSpec(memory_space=pl.ANY)

    out_t = pl.pallas_call(
        _kernel,
        out_shape=jax.ShapeDtypeStruct((D, S), jnp.bfloat16),
        in_specs=[vm, hbm, hbm, hbm, hbm, hbm, vm, vm, vm, vm, vm, vm],
        out_specs=vm,
        scratch_shapes=[
            pltpu.VMEM((NA, NB, 2 * KP), jnp.float32),
            pltpu.VMEM((2 * NB, NA * KP), jnp.bfloat16),
            pltpu.VMEM((S, D), jnp.bfloat16),
            pltpu.VMEM((S, D), jnp.bfloat16),
            pltpu.VMEM((DF, S), jnp.bfloat16),
            pltpu.VMEM((DF, S), jnp.bfloat16),
            pltpu.VMEM((NB, NA, KP), jnp.float32),
            pltpu.VMEM((NB, NA, KP), jnp.float32),
            pltpu.VMEM((D, F), jnp.bfloat16),
            pltpu.VMEM((D, F), jnp.bfloat16),
            pltpu.VMEM((D, F), jnp.bfloat16),
            pltpu.VMEM((F, D), jnp.bfloat16),
            pltpu.SemaphoreType.DMA((5,)),
        ],
        compiler_params=pltpu.CompilerParams(vmem_limit_bytes=100 * 1024 * 1024),
    )(xt, A_w_r.T, A_w_i.T, B_w_gate, B_w_up, B_w_down.T, fd, ff, fv, twr, twi, g)
    return out_t.T.reshape(1, S, D)
```

```python
import math

import numpy as np
import jax
import jax.numpy as jnp
import jax.experimental.pallas as pl
import jax.experimental.pallas.tpu as pltpu

S = 2048
D = 448
F = 1792
DF = D // 2 + 1
KP = 256
NA = 16
NB = 128
EPS = 1e-5
FFN_ROWS = 512


def _constants():
    d = np.arange(D)[:, None].astype(np.float64)
    k = np.arange(KP)[None, :].astype(np.float64)
    valid = (np.arange(KP) < DF)[None, :]
    ang = 2.0 * np.pi * d * k / D
    fd = np.concatenate(
        [np.where(valid, np.cos(ang), 0.0), np.where(valid, -np.sin(ang), 0.0)], axis=1
    )

    b = np.arange(NB).astype(np.float64)
    angb = 2.0 * np.pi * b[:, None] * b[None, :] / NB
    fr, fi = np.cos(angb), -np.sin(angb)
    ff = np.block([[fr, -fi], [fi, fr]])
    fv = np.block([[fr, fi], [-fi, fr]])

    fa = np.arange(NA).astype(np.float64)
    angt = 2.0 * np.pi * b[None, :] * fa[:, None] / S
    twr = np.broadcast_to(np.cos(angt)[:, :, None], (NA, NB, 128)).copy()
    twi = np.broadcast_to(-np.sin(angt)[:, :, None], (NA, NB, 128)).copy()

    ck = np.where((np.arange(KP) == 0) | (np.arange(KP) == D // 2), 1.0, 2.0)
    ck = np.where(np.arange(KP) < DF, ck, 0.0)[:, None]
    scale = 1.0 / (D * S)
    angg = 2.0 * np.pi * np.arange(KP)[:, None] * np.arange(D)[None, :] / D
    g = np.concatenate([ck * np.cos(angg) * scale, -ck * np.sin(angg) * scale], axis=0)

    return (
        jnp.asarray(fd, jnp.bfloat16),
        jnp.asarray(ff, jnp.bfloat16),
        jnp.asarray(fv, jnp.bfloat16),
        jnp.asarray(twr, jnp.float32),
        jnp.asarray(twi, jnp.float32),
        jnp.asarray(g, jnp.bfloat16),
    )


def _cmul_const(re, im, c, s):
    if abs(c - 1.0) < 1e-12 and abs(s) < 1e-12:
        return re, im
    if abs(c + 1.0) < 1e-12 and abs(s) < 1e-12:
        return -re, -im
    if abs(c) < 1e-12 and abs(s + 1.0) < 1e-12:
        return im, -re
    if abs(c) < 1e-12 and abs(s - 1.0) < 1e-12:
        return -im, re
    return re * c - im * s, re * s + im * c


def _fft_list(xs, sign):
    n = len(xs)
    if n == 1:
        return xs
    ev = _fft_list(xs[0::2], sign)
    od = _fft_list(xs[1::2], sign)
    out = [None] * n
    for k in range(n // 2):
        ang = sign * 2.0 * math.pi * k / n
        tr, ti = _cmul_const(od[k][0], od[k][1], math.cos(ang), math.sin(ang))
        out[k] = (ev[k][0] + tr, ev[k][1] + ti)
        out[k + n // 2] = (ev[k][0] - tr, ev[k][1] - ti)
    return out


def _layernorm(v):
    mu = jnp.mean(v, axis=-1, keepdims=True)
    c = v - mu
    var = jnp.mean(c * c, axis=-1, keepdims=True)
    return c * jax.lax.rsqrt(var + EPS)


def _kernel(xt_ref, wrt_hbm, wit_hbm, wg_hbm, wu_hbm, wdt_hbm, fd_ref, ff_ref, fv_ref,
            twr_ref, twi_ref, g_ref, o_ref,
            z_ref, t_ref, x_ref, h_ref, wtr_ref, wti_ref, wr_ref, wi_ref, wg_ref, wu_ref, wdt_ref,
            wd_ref, v_ref, sems):
    f32 = jnp.float32
    bf16 = jnp.bfloat16

    copies = [
        pltpu.make_async_copy(wrt_hbm, wtr_ref, sems.at[0]),
        pltpu.make_async_copy(wit_hbm, wti_ref, sems.at[1]),
        pltpu.make_async_copy(wg_hbm, wg_ref, sems.at[2]),
        pltpu.make_async_copy(wu_hbm, wu_ref, sems.at[3]),
        pltpu.make_async_copy(wdt_hbm, wdt_ref, sems.at[4]),
    ]
    for c in copies:
        c.start()

    x_ref[...] = xt_ref[...].T

    xn = _layernorm(x_ref[...].astype(f32)).astype(bf16)
    z_ref[...] = jnp.dot(xn, fd_ref[...], preferred_element_type=f32)

    CH = 32
    for ch in range(NB // CH):
        r0 = ch * CH
        xs = [(z_ref[a * NB + r0:a * NB + r0 + CH, 0:KP], z_ref[a * NB + r0:a * NB + r0 + CH, KP:2 * KP])
              for a in range(NA)]
        ys = _fft_list(xs, -1.0)
        for fa in range(NA):
            re, im = ys[fa]
            if fa > 0:
                c = jnp.concatenate([twr_ref[fa, r0:r0 + CH, :]] * 2, axis=1)
                s = jnp.concatenate([twi_ref[fa, r0:r0 + CH, :]] * 2, axis=1)
                re, im = re * c - im * s, re * s + im * c
            t_ref[r0:r0 + CH, fa * KP:(fa + 1) * KP] = re.astype(bf16)
            t_ref[NB + r0:NB + r0 + CH, fa * KP:(fa + 1) * KP] = im.astype(bf16)

    xx = jnp.dot(ff_ref[...], t_ref[...], preferred_element_type=f32)
    copies[0].wait()
    copies[1].wait()
    zpad = jnp.zeros((KP - DF, S), f32)
    wr_full = jnp.concatenate([wtr_ref[...].astype(f32), zpad], axis=0).T
    wi_full = jnp.concatenate([wti_ref[...].astype(f32), zpad], axis=0).T
    for j in range(2):
        wr_ref[j] = wr_full[:, j * 128:(j + 1) * 128]
        wi_ref[j] = wi_full[:, j * 128:(j + 1) * 128]
    for fa in range(NA):
        xr = xx[0:NB, fa * KP:(fa + 1) * KP]
        xi = xx[NB:2 * NB, fa * KP:(fa + 1) * KP]
        wr = jnp.concatenate([wr_ref[j, pl.ds(fa, NB, stride=NA), :] for j in range(2)], axis=1)
        wi = jnp.concatenate([wi_ref[j, pl.ds(fa, NB, stride=NA), :] for j in range(2)], axis=1)
        t_ref[0:NB, fa * KP:(fa + 1) * KP] = (xr * wr - xi * wi).astype(bf16)
        t_ref[NB:2 * NB, fa * KP:(fa + 1) * KP] = (xr * wi + xi * wr).astype(bf16)
    uu = jnp.dot(fv_ref[...], t_ref[...], preferred_element_type=f32)

    for ch in range(NB // CH):
        r0 = ch * CH
        xs = []
        for fa in range(NA):
            re = uu[r0:r0 + CH, fa * KP:(fa + 1) * KP]
            im = uu[NB + r0:NB + r0 + CH, fa * KP:(fa + 1) * KP]
            if fa > 0:
                c = jnp.concatenate([twr_ref[fa, r0:r0 + CH, :]] * 2, axis=1)
                s = jnp.concatenate([twi_ref[fa, r0:r0 + CH, :]] * 2, axis=1)
                re, im = re * c + im * s, im * c - re * s
            xs.append((re, im))
        vs = _fft_list(xs, 1.0)
        for a in range(NA):
            v_ref[a * NB + r0:a * NB + r0 + CH, :] = jnp.concatenate(
                [vs[a][0], vs[a][1]], axis=1).astype(bf16)

    y = jnp.dot(v_ref[...], g_ref[...], preferred_element_type=f32).astype(bf16)
    h_ref[...] = x_ref[...] + y

    copies[2].wait()
    copies[3].wait()
    copies[4].wait()
    wd_ref[...] = wdt_ref[...].T

    for r in range(S // FFN_ROWS):
        h = h_ref[r * FFN_ROWS:(r + 1) * FFN_ROWS, :]
        hn = _layernorm(h.astype(f32)).astype(bf16)
        gg = jnp.dot(hn, wg_ref[...], preferred_element_type=f32).astype(bf16)
        up = jnp.dot(hn, wu_ref[...], preferred_element_type=f32).astype(bf16)
        hh = gg * up
        out = jnp.dot(hh, wd_ref[...], preferred_element_type=f32).astype(bf16)
        o_ref[:, r * FFN_ROWS:(r + 1) * FFN_ROWS] = (h + out).T


@jax.jit
def pallas_sequential_preLN__spectral_gfnet__glu_gated_bilinear__prompt_kernel(
    A_x: jax.Array,
    A_w_r: jax.Array,
    A_w_i: jax.Array,
    B_x: jax.Array,
    B_w_gate: jax.Array,
    B_w_up: jax.Array,
    B_w_down: jax.Array,
):
    xt = A_x.reshape(S, D).T
    fd, ff, fv, twr, twi, g = _constants()
    vm = pl.BlockSpec(memory_space=pltpu.VMEM)
    hbm = pl.BlockSpec(memory_space=pl.ANY)

    out_t = pl.pallas_call(
        _kernel,
        out_shape=jax.ShapeDtypeStruct((D, S), jnp.bfloat16),
        in_specs=[vm, hbm, hbm, hbm, hbm, hbm, vm, vm, vm, vm, vm, vm],
        out_specs=vm,
        scratch_shapes=[
            pltpu.VMEM((S, 2 * KP), jnp.float32),
            pltpu.VMEM((2 * NB, NA * KP), jnp.bfloat16),
            pltpu.VMEM((S, D), jnp.bfloat16),
            pltpu.VMEM((S, D), jnp.bfloat16),
            pltpu.VMEM((DF, S), jnp.bfloat16),
            pltpu.VMEM((DF, S), jnp.bfloat16),
            pltpu.VMEM((2, S, 128), jnp.float32),
            pltpu.VMEM((2, S, 128), jnp.float32),
            pltpu.VMEM((D, F), jnp.bfloat16),
            pltpu.VMEM((D, F), jnp.bfloat16),
            pltpu.VMEM((D, F), jnp.bfloat16),
            pltpu.VMEM((F, D), jnp.bfloat16),
            pltpu.VMEM((S, 2 * KP), jnp.bfloat16),
            pltpu.SemaphoreType.DMA((5,)),
        ],
        compiler_params=pltpu.CompilerParams(vmem_limit_bytes=100 * 1024 * 1024),
    )(xt, A_w_r.T, A_w_i.T, B_w_gate, B_w_up, B_w_down.T, fd, ff, fv, twr, twi, g)
    return out_t.T.reshape(1, S, D)
```
